```python
import os as _os
_os.environ.setdefault("JAX_PLATFORMS", "cpu")
import jax
import jax.numpy as jnp

def _softmax(x, axis=-1):
    return jax.nn.softmax(x, axis=axis)
def _gelu(x):
    return jax.nn.gelu(x, approximate=True)
def _silu(x):
    return jax.nn.silu(x)
def _sigmoid(x):
    return jax.nn.sigmoid(x)
def _layernorm(x, axis=-1, eps=1e-5):
    m = jnp.mean(x, axis=axis, keepdims=True)
    v = jnp.var(x, axis=axis, keepdims=True)
    return (x - m) / jnp.sqrt(v + eps)
def _scatter_add(tgt, idx, src, axis=0):
    return tgt.at[idx].add(src)
def _segment_sum(src, seg, n):
    return jax.ops.segment_sum(src, seg, n)
class _Rng:
    def __init__(self, key):
        self._k = key
    def _next(self):
        self._k, sub = jax.random.split(self._k)
        return sub
    def normal(self, shape):
        return jax.random.normal(self._next(), shape, dtype=jnp.bfloat16)
    def randint(self, lo, hi, shape):
        return jax.random.randint(self._next(), shape, lo, hi, dtype=jnp.int32)
    def uniform(self, shape, lo=0.0, hi=1.0):
        return jax.random.uniform(self._next(), shape, jnp.bfloat16, lo, hi)
    def permutation(self, n):
        return jax.random.permutation(self._next(), n)


kernel_name = 'sequential_preLN__softmax_full_mha__dense_activation_gelu__prompt'

def setup_inputs():
    _rng = _Rng(jax.random.key(int.from_bytes(__import__("os").urandom(4), "little")))
    _w = (lambda a: (lambda t: t.astype(jnp.bfloat16) if jnp.issubdtype(t.dtype, jnp.floating) else t)(jnp.asarray(a)))
    def _A_setup():
        B, S, D = 1, 2048, 640
        return {
            "x": _w((lambda *s: _rng.normal(s) * 0.05)(B, S, D)),
            "wqkv": _w((lambda *s: _rng.normal(s) * 0.05)(D, 3 * D)),
            "wo": _w((lambda *s: _rng.normal(s) * 0.05)(D, D)),
        }
    _A_in = _A_setup()

    def _B_setup():
        B, S, D, F = 1, 2048, 640, 1536
        return {
            "x": _w((lambda *s: _rng.normal(s) * 0.05)(B, S, D)),
            "w1": _w((lambda *s: _rng.normal(s) * 0.4)(D, F) * (D ** -0.5)),
            "b1": _w((lambda *s: _rng.normal(s) * 0.4)(F) * 0.01),
            "w2": _w((lambda *s: _rng.normal(s) * 0.4)(F, D) * (F ** -0.5)),
            "b2": _w((lambda *s: _rng.normal(s) * 0.05)(D) * 0.01),
        }
    _B_in = _B_setup()

    return {
        "A_x": _A_in["x"],
        "A_wqkv": _A_in["wqkv"],
        "A_wo": _A_in["wo"],
        "B_x": _B_in["x"],
        "B_w1": _B_in["w1"],
        "B_b1": _B_in["b1"],
        "B_w2": _B_in["w2"],
        "B_b2": _B_in["b2"],
    }

def reference(A_x, A_wqkv, A_wo, B_x, B_w1, B_b1, B_w2, B_b2):
    def _A_ref(x, wqkv, wo):
        B, S, D = x.shape
        H = 32; Dh = D // H
        qkv = (lambda x, *d: x.transpose(*d))((x @ wqkv).reshape(B, S, 3, H, Dh), 2, 0, 3, 1, 4)
        q, k, v = qkv[0], qkv[1], qkv[2]
        scale = Dh ** -0.5
        scores = jnp.einsum("bhqd,bhkd->bhqk", q, k) * scale
        p = _softmax(scores, axis=-1)
        o = jnp.einsum("bhqk,bhkd->bhqd", p, v)
        return (lambda x, *d: x.transpose(*d))(o, 0, 2, 1, 3).reshape(B, S, D) @ wo

    def _B_ref(x, w1, b1, w2, b2):
        h = jnp.einsum("bsd,df->bsf", x, w1) + b1
        h = _gelu(h)
        return jnp.einsum("bsf,fd->bsd", h, w2) + b2

    x = A_x
    h = x + _A_ref(_layernorm(x, axis=-1), A_wqkv, A_wo)
    h2 = h + _B_ref(_layernorm(h, axis=-1), B_w1, B_b1, B_w2, B_b2)
    return h2
```

```python
import math

import jax
import jax.numpy as jnp
import jax.experimental.pallas as pl
import jax.experimental.pallas.tpu as pltpu
from jax import lax

H = 32
TQ = 128
RB = 256
EPS = 1e-5
NT = (((1,), (1,)), ((), ()))


def _ln(x):
    m = jnp.mean(x, axis=-1, keepdims=True)
    c = x - m
    v = jnp.mean(c * c, axis=-1, keepdims=True)
    return c * lax.rsqrt(v + EPS)


def _gelu(x):
    k0 = math.sqrt(2.0 / math.pi)
    return 0.5 * x * (1.0 + jnp.tanh(k0 * (x + 0.044715 * (x * x * x))))


def _kernel(x_ref, wqkv_ref, wo_ref, w1_ref, b1_ref, w2_ref, b2_ref, o_ref,
            q_s, k_s, vt_s, ot_s):
    S, D = x_ref.shape
    dh = D // H
    gw = 6 * dh
    ng = (D + gw - 1) // gw
    i = pl.program_id(0)
    f32, bf16 = jnp.float32, jnp.bfloat16

    def regroup(y):
        parts = []
        for g in range(ng):
            a, b = g * gw, min((g + 1) * gw, D)
            parts += [y[:, a:b], jnp.zeros((y.shape[0], 128 - (b - a)), y.dtype)]
        return jnp.concatenate(parts, axis=1)

    @pl.when(i == 0)
    def _():
        wvt = wqkv_ref[:, 2 * D:].astype(f32).T.astype(bf16)

        def body(r, c):
            rows = pl.ds(pl.multiple_of(r * RB, RB), RB)
            xn = _ln(x_ref[rows, :].astype(f32)).astype(bf16)
            qk = jnp.dot(xn, wqkv_ref[:, :2 * D], preferred_element_type=f32)
            q = qk[:, :D] * (dh ** -0.5 * math.log2(math.e))
            q_s[rows, :] = regroup(q).astype(bf16)
            k_s[rows, :] = regroup(qk[:, D:]).astype(bf16)
            vt = lax.dot_general(wvt, xn, NT, preferred_element_type=f32)
            row = lax.broadcasted_iota(jnp.int32, (24, RB), 0)
            for p in range(H // 2):
                vt_s[2 * p, :, rows] = jnp.where(row < 20, vt[40 * p:40 * p + 24], 1.0)
                vt_s[2 * p + 1, :, rows] = jnp.where(row >= 4, vt[40 * p + 16:40 * p + 40], 1.0)
            return c

        lax.fori_loop(0, S // RB, body, 0)

    qrows = pl.ds(pl.multiple_of(i * TQ, TQ), TQ)
    lane = lax.broadcasted_iota(jnp.int32, (TQ, 128), 1)
    row = lax.broadcasted_iota(jnp.int32, (8, TQ), 0)

    def pair(p, c):
        g = p // 3
        lanes = pl.ds(pl.multiple_of(g * 128, 128), 128)
        qg = q_s[qrows, lanes].astype(f32)
        outs = []
        for e in range(2):
            lo = ((p % 3) * 2 + e) * dh
            qm = jnp.where((lane >= lo) & (lane < lo + dh), qg, 0.0).astype(bf16)
            st = lax.dot_general(k_s[:, lanes], qm, NT, preferred_element_type=f32)
            m = jnp.max(st, axis=0, keepdims=True)
            pt = jnp.exp2(st - m).astype(bf16)
            ot = jnp.dot(vt_s[2 * p + e].astype(bf16), pt, preferred_element_type=f32)
            l = ot[23:24] if e == 0 else ot[0:1]
            outs.append(ot / l)
        mid = jnp.where(row < 4, outs[0][16:24], outs[1][0:8])
        ot_s[pl.ds(pl.multiple_of(p * 40, 8), 40), :] = jnp.concatenate(
            [outs[0][:16], mid, outs[1][8:]], axis=0)
        return c

    lax.fori_loop(0, H // 2, pair, 0)

    o = ot_s[...].T.astype(bf16)
    h = x_ref[qrows, :].astype(f32) + jnp.dot(o, wo_ref[...], preferred_element_type=f32)
    hn = _ln(h).astype(bf16)
    a = jnp.dot(hn, w1_ref[...], preferred_element_type=f32) + b1_ref[...].astype(f32)
    a = _gelu(a).astype(bf16)
    y = jnp.dot(a, w2_ref[...], preferred_element_type=f32) + b2_ref[...].astype(f32)
    o_ref[...] = (h + y).astype(o_ref.dtype)


@jax.jit
def pallas_sequential_preLN__softmax_full_mha__dense_activation_gelu__prompt_kernel(
    A_x: jax.Array,
    A_wqkv: jax.Array,
    A_wo: jax.Array,
    B_x: jax.Array,
    B_w1: jax.Array,
    B_b1: jax.Array,
    B_w2: jax.Array,
    B_b2: jax.Array,
):
    del B_x
    B, S, D = A_x.shape
    F = B_w1.shape[1]
    assert B == 1
    full = lambda *s: pl.BlockSpec(s, lambda i: (0,) * len(s))
    out = pl.pallas_call(
        _kernel,
        grid=(S // TQ,),
        in_specs=[full(S, D), full(D, 3 * D), full(D, D), full(D, F), full(1, F),
                  full(F, D), full(1, D)],
        out_specs=pl.BlockSpec((TQ, D), lambda i: (i, 0)),
        out_shape=jax.ShapeDtypeStruct((S, D), A_x.dtype),
        scratch_shapes=[
            pltpu.VMEM((S, 768), jnp.bfloat16),
            pltpu.VMEM((S, 768), jnp.bfloat16),
            pltpu.VMEM((H, 24, S), jnp.float32),
            pltpu.VMEM((D, TQ), jnp.float32),
        ],
        compiler_params=pltpu.CompilerParams(
            dimension_semantics=("arbitrary",),
            vmem_limit_bytes=100 * 1024 * 1024,
        ),
    )(A_x.reshape(S, D), A_wqkv, A_wo, B_w1, B_b1.reshape(1, F), B_w2, B_b2.reshape(1, D))
    return out.reshape(B, S, D)
```

```python
import math

import jax
import jax.numpy as jnp
import jax.experimental.pallas as pl
import jax.experimental.pallas.tpu as pltpu
from jax import lax

H = 32
KC = 128
TQ = 512
RB = 256
LAG = 2
UN = 5
PDT = jnp.bfloat16
EPS = 1e-5
NT = (((1,), (1,)), ((), ()))


def _ln(x):
    m = jnp.mean(x, axis=-1, keepdims=True)
    c = x - m
    v = jnp.mean(c * c, axis=-1, keepdims=True)
    return c * lax.rsqrt(v + EPS)


def _gelu(x):
    k0 = math.sqrt(2.0 / math.pi)
    return 0.5 * x * (1.0 + jnp.tanh(k0 * (x + 0.044715 * (x * x * x))))


def _kernel(x_hbm, wqkv_hbm, wo_hbm, w1_hbm, b1_ref, w2_hbm, b2_ref, o_ref,
            qt_s, k_s, vt_s, ot_s, s0_s, s1_s, wo_ref, w1_ref, w2_ref, sems,
            x_ref, wqkv_ref, wsem, xsem):
    S, D = x_ref.shape
    dh = D // H
    gw = 6 * dh
    ng = (D + gw - 1) // gw
    i = pl.program_id(0)
    f32, bf16 = jnp.float32, jnp.bfloat16

    late = [pltpu.make_async_copy(a, b, sems.at[n]) for n, (a, b) in enumerate(
        ((wo_hbm, wo_ref), (w1_hbm, w1_ref), (w2_hbm, w2_ref)))]

    @pl.when(i == 0)
    def _():
        def wcp(n):
            cols = pl.ds(n * D, D)
            return pltpu.make_async_copy(wqkv_hbm.at[:, cols], wqkv_ref.at[:, cols], wsem.at[n])

        def xcp(r, rows):
            return pltpu.make_async_copy(x_hbm.at[rows], x_ref.at[rows], xsem.at[r])

        wcp(0).start()
        wcp(2).start()
        xcp(0, pl.ds(0, RB)).start()
        wcp(1).start()
        wcp(0).wait()
        wqt = wqkv_ref[:, :D].astype(f32).T.astype(bf16)
        wcp(2).wait()
        wvt = wqkv_ref[:, 2 * D:].astype(f32).T.astype(bf16)
        qt_s[D:, :] = jnp.zeros((qt_s.shape[0] - D, S), f32)
        wcp(1).wait()
        for r in range(1, S // RB):
            xcp(r, pl.ds(r * RB, RB)).start()
        for cp in late:
            cp.start()

        def body(r, c):
            rows = pl.ds(pl.multiple_of(r * RB, RB), RB)
            xcp(r, rows).wait()
            xn = _ln(x_ref[rows, :].astype(f32)).astype(bf16)
            k = jnp.dot(xn, wqkv_ref[:, D:2 * D], preferred_element_type=f32)
            for g in range(ng):
                a, b = g * gw, min((g + 1) * gw, D)
                k_s[g, rows, :] = jnp.concatenate(
                    [k[:, a:b], jnp.zeros((RB, 128 - (b - a)), f32)], axis=1).astype(bf16)
            qt = lax.dot_general(wqt, xn, NT, preferred_element_type=f32)
            qt_s[:D, rows] = qt * (dh ** -0.5 * math.log2(math.e))
            vt = lax.dot_general(wvt, xn, NT, preferred_element_type=f32)
            row = lax.broadcasted_iota(jnp.int32, (24, RB), 0)
            for p in range(H // 2):
                va = jnp.where(row < 20, vt[40 * p:40 * p + 24], 1.0)
                vb = jnp.where(row >= 4, vt[40 * p + 16:40 * p + 40], 1.0)
                vt_s[2 * p, :, rows] = va
                vt_s[2 * p + 1, :, rows] = vb
            return c

        lax.fori_loop(0, S // RB, body, 0)
        for cp in late:
            cp.wait()

    qcols = pl.ds(pl.multiple_of(i * TQ, TQ), TQ)
    r128 = lax.broadcasted_iota(jnp.int32, (128, TQ), 0)
    r8 = lax.broadcasted_iota(jnp.int32, (8, TQ), 0)

    def q_of(h):
        g = h // 6
        lo = (h - g * 6) * dh
        q = qt_s[pl.ds(pl.multiple_of(g * gw, 8), 128), qcols]
        return g, jnp.where((r128 >= lo) & (r128 < lo + dh), q, 0.0).astype(bf16)

    def stage(h_qk, s_qk, h_pv, s_pv, m_pv):
        m = acc = None
        if h_qk is not None:
            g, q = q_of(h_qk)
        for c in range(S // KC + LAG):
            ks = slice(c * KC, (c + 1) * KC)
            if h_qk is not None and c < S // KC:
                st = jnp.dot(k_s[g, ks, :], q, preferred_element_type=f32)
                s_qk[ks, :] = st
                mc = jnp.max(st.reshape(KC // 8, 8, TQ), axis=0)
                m = mc if m is None else jnp.maximum(m, mc)
            if h_pv is not None and c >= LAG:
                ks = slice((c - LAG) * KC, (c - LAG + 1) * KC)
                pt = jnp.exp2(s_pv[ks, :] - m_pv).astype(PDT)
                a = jnp.dot(vt_s[h_pv, :, ks], pt, preferred_element_type=f32)
                acc = a if acc is None else acc + a
        if m is not None:
            m = jnp.max(m, axis=0, keepdims=True)
        return m, acc

    def pair(p, m0, last=False):
        m1, oa = stage(2 * p + 1, s1_s, 2 * p, s0_s, m0)
        m2, ob = stage(None if last else 2 * p + 2, s0_s, 2 * p + 1, s1_s, m1)
        oa = oa / oa[23:24]
        ob = ob / ob[0:1]
        mid = jnp.where(r8 < 4, oa[16:24], ob[0:8])
        ot_s[pl.ds(pl.multiple_of(p * 40, 8), 40), :] = jnp.concatenate(
            [oa[:16], mid, ob[8:]], axis=0)
        return m2

    m0, _ = stage(0, s0_s, None, None, None)
    m0 = lax.fori_loop(0, H // 2 - 1, pair, m0, unroll=UN)
    pair(H // 2 - 1, m0, last=True)

    o = ot_s[...].T.astype(bf16)
    h = x_ref[qcols, :].astype(f32) + jnp.dot(o, wo_ref[...], preferred_element_type=f32)
    hn = _ln(h).astype(bf16)
    a = jnp.dot(hn, w1_ref[...], preferred_element_type=f32) + b1_ref[...].astype(f32)[None, :]
    a = _gelu(a).astype(bf16)
    y = jnp.dot(a, w2_ref[...], preferred_element_type=f32) + b2_ref[...].astype(f32)[None, :]
    o_ref[...] = (h + y).astype(o_ref.dtype)


@jax.jit
def pallas_sequential_preLN__softmax_full_mha__dense_activation_gelu__prompt_kernel(
    A_x: jax.Array,
    A_wqkv: jax.Array,
    A_wo: jax.Array,
    B_x: jax.Array,
    B_w1: jax.Array,
    B_b1: jax.Array,
    B_w2: jax.Array,
    B_b2: jax.Array,
):
    del B_x
    B, S, D = A_x.shape
    F = B_w1.shape[1]
    assert B == 1
    full = lambda *s: pl.BlockSpec(s, lambda i: (0,) * len(s))
    hbm = pl.BlockSpec(memory_space=pl.ANY)
    out = pl.pallas_call(
        _kernel,
        grid=(S // TQ,),
        in_specs=[hbm, hbm, hbm, hbm, full(F), hbm, full(D)],
        out_specs=pl.BlockSpec((TQ, D), lambda i: (i, 0)),
        out_shape=jax.ShapeDtypeStruct((S, D), A_x.dtype),
        scratch_shapes=[
            pltpu.VMEM((728, S), jnp.float32),
            pltpu.VMEM((6, S, 128), jnp.bfloat16),
            pltpu.VMEM((H, 24, S), jnp.float32),
            pltpu.VMEM((D, TQ), jnp.float32),
            pltpu.VMEM((S, TQ), jnp.float32),
            pltpu.VMEM((S, TQ), jnp.float32),
            pltpu.VMEM((D, D), jnp.bfloat16),
            pltpu.VMEM((D, F), jnp.bfloat16),
            pltpu.VMEM((F, D), jnp.bfloat16),
            pltpu.SemaphoreType.DMA((3,)),
            pltpu.VMEM((S, D), jnp.bfloat16),
            pltpu.VMEM((D, 3 * D), jnp.bfloat16),
            pltpu.SemaphoreType.DMA((3,)),
            pltpu.SemaphoreType.DMA((S // RB,)),
        ],
        compiler_params=pltpu.CompilerParams(
            dimension_semantics=("arbitrary",),
            vmem_limit_bytes=100 * 1024 * 1024,
        ),
    )(A_x.reshape(S, D), A_wqkv, A_wo, B_w1, B_b1, B_w2, B_b2)
    return out.reshape(B, S, D)
```
